```python
import jax
import jax.numpy as jnp

def _softmax(x, axis=-1):
    return jax.nn.softmax(x, axis=axis)
def _gelu(x):
    return jax.nn.gelu(x, approximate=True)
def _silu(x):
    return jax.nn.silu(x)
def _sigmoid(x):
    return jax.nn.sigmoid(x)
def _layernorm(x, axis=-1, eps=1e-5):
    m = jnp.mean(x, axis=axis, keepdims=True)
    v = jnp.var(x, axis=axis, keepdims=True)
    return (x - m) / jnp.sqrt(v + eps)
def _scatter_add(tgt, idx, src, axis=0):
    return tgt.at[idx].add(src)
def _segment_sum(src, seg, n):
    return jax.ops.segment_sum(src, seg, n)
class _Rng:
    def __init__(self, key):
        self._k = key
    def _next(self):
        self._k, sub = jax.random.split(self._k)
        return sub
    def normal(self, shape):
        return jax.random.normal(self._next(), shape, dtype=jnp.bfloat16)
    def randint(self, lo, hi, shape):
        return jax.random.randint(self._next(), shape, lo, hi, dtype=jnp.int32)
    def uniform(self, shape, lo=0.0, hi=1.0):
        return jax.random.uniform(self._next(), shape, jnp.bfloat16, lo, hi)
    def permutation(self, n):
        return jax.random.permutation(self._next(), n)


kernel_name = 'interleave_layers__sliding_block__sliding_local_dilated__prompt'

def setup_inputs():
    _rng = _Rng(jax.random.key(int.from_bytes(__import__("os").urandom(4), "little")))
    _w = (lambda a: (lambda t: t.astype(jnp.bfloat16) if jnp.issubdtype(t.dtype, jnp.floating) else t)(jnp.asarray(a)))
    def _A_setup():
        B, S, D = 1, 2048, 1024
        return {
            "x": _w((lambda *s: _rng.normal(s) * 0.05)(B, S, D)),
            "wqkv": _w((lambda *s: _rng.normal(s) * 0.05)(D, 3 * D)),
            "wo": _w((lambda *s: _rng.normal(s) * 0.05)(D, D)),
        }
    _A_in = _A_setup()

    def _B_setup():
        B, S, D = 1, 2048, 1024
        return {
            "x": _w((lambda *s: _rng.normal(s) * 0.05)(B, S, D)),
            "wqkv": _w((lambda *s: _rng.normal(s) * 0.05)(D, 3 * D)),
            "wo": _w((lambda *s: _rng.normal(s) * 0.05)(D, D)),
        }
    _B_in = _B_setup()

    return {
        "A_x": _A_in["x"],
        "A_wqkv": _A_in["wqkv"],
        "A_wo": _A_in["wo"],
        "B_x": _B_in["x"],
        "B_wqkv": _B_in["wqkv"],
        "B_wo": _B_in["wo"],
    }

def reference(A_x, A_wqkv, A_wo, B_x, B_wqkv, B_wo):
    def _A_ref(x, wqkv, wo):
        B, S, D = x.shape
        H = 32; Dh = D // H; W = 256
        qkv = (lambda x, *d: x.transpose(*d))((x @ wqkv).reshape(B, S, 3, H, Dh), 2, 0, 3, 1, 4)
        q, k, v = qkv[0], qkv[1], qkv[2]
        scores = jnp.einsum("bhqd,bhkd->bhqk", q, k) * (Dh ** -0.5)
        idx = jnp.arange(S)
        mask = (idx[:, None] - idx[None, :] >= 0) & (idx[:, None] - idx[None, :] < W)
        scores = jnp.where(mask[None, None], scores, -1e9)
        p = _softmax(scores, axis=-1)
        o = jnp.einsum("bhqk,bhkd->bhqd", p, v)
        return (lambda x, *d: x.transpose(*d))(o, 0, 2, 1, 3).reshape(B, S, D) @ wo

    def _B_ref(x, wqkv, wo):
        B, S, D = x.shape
        H = 32; Dh = D // H
        W, dil = 8, 2
        qkv = (lambda x, *d: x.transpose(*d))((x @ wqkv).reshape(B, S, 3, H, Dh), 2, 0, 3, 1, 4)
        q, k, v = qkv[0], qkv[1], qkv[2]
        scale = Dh ** -0.5
        pos = jnp.arange(S)
        off = jnp.arange(W) * dil
        idx = pos[:, None] - off[None, :]
        mask = idx >= 0
        idx_c = jnp.where(mask, idx, 0).reshape(-1)
        kg = k[:, :, idx_c, :].reshape(B, H, S, W, Dh)
        vg = v[:, :, idx_c, :].reshape(B, H, S, W, Dh)
        logits = jnp.einsum("bhsd,bhswd->bhsw", q, kg) * scale
        logits = jnp.where(mask[None, None, :, :], logits, -1e9)
        attn = _softmax(logits, axis=-1)
        o = jnp.einsum("bhsw,bhswd->bhsd", attn, vg)
        return (lambda x, *d: x.transpose(*d))(o, 0, 2, 1, 3).reshape(B, S, D) @ wo

    x = A_x
    x = x + _A_ref(_layernorm(x, axis=-1), A_wqkv, A_wo)
    x = x + _B_ref(_layernorm(x, axis=-1), B_wqkv, B_wo)
    x = x + _A_ref(_layernorm(x, axis=-1), A_wqkv, A_wo)
    x = x + _B_ref(_layernorm(x, axis=-1), B_wqkv, B_wo)
    return x
```

```python
import math

import jax
import jax.numpy as jnp
import numpy as np
from jax import lax
import jax.experimental.pallas as pl
import jax.experimental.pallas.tpu as pltpu

S = 2048
D = 1024
H = 32
DH = 32
NG = D // 128
TQ = 128
NT = S // TQ
PAD = 256
GA = 2
GB = 4
GM = max(GA, GB)
TC = 512
NC = S // TC
NEG = -1e9
QSCALE = (DH ** -0.5) * math.log2(math.e)
EPS = 1e-5
BF = jnp.bfloat16
F32 = jnp.float32
NT_DIMS = (((1,), (1,)), ((), ()))


def _bias_tables():
    k = np.arange(384)[:, None] - 256
    q = np.arange(128)[None, :]
    a = []
    for t in range(3):
        ok = (q - k >= 0) & (q - k < 256) & (k + t * 128 >= 0)
        a.append(np.where(ok, 0.0, NEG))
    k = np.arange(144)[:, None] - 16
    b = []
    for t in range(2):
        d = q - k
        ok = (d >= 0) & (d <= 14) & (d % 2 == 0) & (k + t * 128 >= 0)
        b.append(np.where(ok, 0.0, NEG))
    return np.stack(a).astype(np.float32), np.stack(b).astype(np.float32)


def _kernel(ba_ref, bb_ref, x_hbm, wa_hbm, woa_hbm, wb_hbm, wob_hbm, out_hbm,
            xin, xr, w, wo, qT, kk, vT, oo, stage,
            sa0, sa1, pa0, pa1, sb0, sb1, pb0, pb1, m0, m1, l0, l1, sem_x, sem_w, sem_o):
    def x_copy(c):
        return pltpu.make_async_copy(x_hbm.at[pl.ds(c * TC, TC)], xin.at[pl.ds(c * TC, TC)], sem_x.at[c])

    w_copies = [
        pltpu.make_async_copy(wa_hbm, w.at[0], sem_w.at[0]),
        pltpu.make_async_copy(woa_hbm, wo.at[0], sem_w.at[1]),
        pltpu.make_async_copy(wb_hbm, w.at[1], sem_w.at[2]),
        pltpu.make_async_copy(wob_hbm, wo.at[1], sem_w.at[3]),
    ]
    x_copy(0).start()
    w_copies[0].start()
    for c in range(1, NC):
        x_copy(c).start()
    for cp in w_copies[1:]:
        cp.start()

    for g in range(NG):
        kk[g, 0:PAD, :] = jnp.zeros((PAD, 128), BF)
        for t in range(PAD // 128):
            vT[t, g] = jnp.zeros((128, 128), BF)

    def project(c, x, wi):
        m = jnp.mean(x, axis=-1, keepdims=True)
        xc = x - m
        v = jnp.mean(xc * xc, axis=-1, keepdims=True)
        ln = (xc * lax.rsqrt(v + EPS)).astype(BF)
        for b in range(D // 512):
            q = jnp.dot(ln, w[wi, :, b * 512:(b + 1) * 512], preferred_element_type=F32)
            q = (q * QSCALE).astype(BF)
            for j in range(4):
                for t in range(TC // 128):
                    qT[c * (TC // 128) + t, b * 4 + j] = q[t * 128:(t + 1) * 128, j * 128:(j + 1) * 128].T
            k = jnp.dot(ln, w[wi, :, D + b * 512:D + (b + 1) * 512], preferred_element_type=F32).astype(BF)
            for j in range(4):
                kk[b * 4 + j, pl.ds(pl.multiple_of(PAD + c * TC, TC // 2), TC), :] = k[:, j * 128:(j + 1) * 128]
            vv = jnp.dot(ln, w[wi, :, 2 * D + b * 512:2 * D + (b + 1) * 512], preferred_element_type=F32).astype(BF)
            for j in range(4):
                for t in range(TC // 128):
                    vT[2 + c * (TC // 128) + t, b * 4 + j] = vv[t * 128:(t + 1) * 128, j * 128:(j + 1) * 128].T

    def masked_q(i, g):
        q4 = qT[i, g]
        z = jnp.zeros((32, 128), BF)
        cols = []
        for h in range(4):
            cols.append(jnp.concatenate([q4[32 * h:32 * h + 32] if hh == h else z for hh in range(4)], axis=0))
        return jnp.concatenate(cols, axis=1)

    def attention(nk, G, bias_ref, Sb, Pb, Mb, Lb):
        is_a = nk == 384
        nb = NT * NG // G
        prow = 0 if is_a else 112

        def qk(j, b, u):
            n = j * G + u
            i, g = n // NG, n % NG
            k4 = kk[g, pl.ds(pl.multiple_of(i * 128 + PAD + 128 - nk, 16), nk), :]
            s = jnp.dot(k4, masked_q(i, g), preferred_element_type=F32)
            bi = jnp.minimum(i, 2 if is_a else 1)
            ms = [None] * 4
            for r in range(0, nk, 8):
                bias = bias_ref[bi, r:r + 8, :]
                for h in range(4):
                    c = s[r:r + 8, h * 128:(h + 1) * 128] + bias
                    Sb[b][u, r:r + 8, h * 128:(h + 1) * 128] = c
                    ms[h] = c if ms[h] is None else jnp.maximum(ms[h], c)
            for h in range(4):
                Mb[b][u, :, h * 128:(h + 1) * 128] = jnp.broadcast_to(
                    jnp.max(ms[h], axis=0, keepdims=True), (8, 128))

        def ex(b, u):
            for h in range(4):
                cs = slice(h * 128, (h + 1) * 128)
                m = Mb[b][u, :, cs]
                l = None
                for r in range(0, nk, 16):
                    pa = jnp.exp2(Sb[b][u, r:r + 8, cs] - m)
                    pb = jnp.exp2(Sb[b][u, r + 8:r + 16, cs] - m)
                    t = pa + pb
                    l = t if l is None else l + t
                    Pb[b][u, prow + r:prow + r + 16, cs] = jnp.concatenate([pa, pb], axis=0).astype(BF)
                Lb[b][u, :, cs] = jnp.broadcast_to(
                    pltpu.reciprocal(jnp.sum(l, axis=0, keepdims=True), approx=False), (8, 128))

        def pv(j, b, u):
            n = j * G + u
            i, g = n // NG, n % NG
            t0, npr = (0, 384) if is_a else (1, 256)
            outs = []
            for h in range(4):
                cs = slice(h * 128, (h + 1) * 128)
                vt = jnp.concatenate([vT[i + t, g, 32 * h:32 * h + 32, :] for t in range(t0, 3)], axis=1)
                o = jnp.dot(vt, Pb[b][u, 0:npr, cs], preferred_element_type=F32)
                outs.append(o * Lb[b][u, 0:1, cs])
            oo[g, pl.ds(pl.multiple_of(i * 128, 128), 128), :] = jnp.concatenate(outs, axis=0).astype(BF).T

        if not is_a:
            for b in range(2):
                for u in range(G):
                    Pb[b][u, 0:prow, :] = jnp.zeros((prow, 512), BF)

        def step(j, b, p=True, e=True, q=True):
            for u in range(G):
                if p:
                    pv(j - 1, 1 - b, u)
                if e:
                    ex(b, u)
                if q:
                    qk(j + 1, 1 - b, u)

        step(-1, 1, p=False, e=False)
        step(0, 0, p=False)

        def body(j, _):
            pl.when(j % 2 == 1)(lambda: step(j, 1))
            pl.when(j % 2 == 0)(lambda: step(j, 0))
            return 0
        lax.fori_loop(1, nb - 1, body, 0)
        step(nb - 1, 1, q=False)
        step(nb, 0, e=False, q=False)

    def attn_a():
        attention(384, GA, ba_ref, (sa0, sa1), (pa0, pa1), (m0, m1), (l0, l1))

    def attn_b():
        attention(144, GB, bb_ref, (sb0, sb1), (pb0, pb1), (m0, m1), (l0, l1))

    def outproj(c, wi):
        r0 = pl.multiple_of(c * TC, TC)
        o = jnp.concatenate([oo[g, pl.ds(r0, TC), :] for g in range(NG)], axis=1)
        return xr[pl.ds(r0, TC), :] + jnp.dot(o, wo[wi], preferred_element_type=F32)

    w_copies[0].wait()

    def first(c, _):
        x_copy(c).wait()
        r0 = pl.multiple_of(c * TC, TC)
        x = xin[pl.ds(r0, TC), :].astype(F32)
        xr[pl.ds(r0, TC), :] = x
        project(c, x, 0)
        return 0
    lax.fori_loop(0, NC, first, 0)
    for cp in w_copies[1:]:
        cp.wait()

    def mid(wi):
        def body(c, _):
            x = outproj(c, wi)
            xr[pl.ds(pl.multiple_of(c * TC, TC), TC), :] = x
            project(c, x, 1 - wi)
            return 0
        return body

    def pair(p, _):
        attn_a()
        lax.fori_loop(0, NC, mid(0), 0)
        attn_b()

        @pl.when(p == 0)
        def _():
            lax.fori_loop(0, NC, mid(1), 0)
        return 0
    lax.fori_loop(0, 2, pair, 0)

    def out_copy(c):
        return pltpu.make_async_copy(stage.at[c], out_hbm.at[pl.ds(c * TC, TC)], sem_o.at[c])

    def last(c, _):
        stage[c] = outproj(c, 1).astype(BF)
        out_copy(c).start()
        return 0
    lax.fori_loop(0, NC, last, 0)
    for c in range(NC):
        out_copy(c).wait()


@jax.jit
def pallas_interleave_layers__sliding_block__sliding_local_dilated__prompt_kernel(
    A_x, A_wqkv, A_wo, B_x, B_wqkv, B_wo,
):
    ba, bb = _bias_tables()
    any_spec = pl.BlockSpec(memory_space=pl.ANY)
    vm = pl.BlockSpec(memory_space=pltpu.VMEM)
    out = pl.pallas_call(
        _kernel,
        out_shape=jax.ShapeDtypeStruct((S, D), BF),
        in_specs=[vm, vm] + [any_spec] * 5,
        out_specs=any_spec,
        scratch_shapes=[
            pltpu.VMEM((S, D), BF),
            pltpu.VMEM((S, D), F32),
            pltpu.VMEM((2, D, 3 * D), BF),
            pltpu.VMEM((2, D, D), BF),
            pltpu.VMEM((NT, NG, 128, 128), BF),
            pltpu.VMEM((NG, S + PAD, 128), BF),
            pltpu.VMEM((NT + 2, NG, 128, 128), BF),
            pltpu.VMEM((NG, S, 128), BF),
            pltpu.VMEM((NC, TC, D), BF),
            pltpu.VMEM((GA, 384, 512), F32), pltpu.VMEM((GA, 384, 512), F32),
            pltpu.VMEM((GA, 384, 512), BF), pltpu.VMEM((GA, 384, 512), BF),
            pltpu.VMEM((GB, 144, 512), F32), pltpu.VMEM((GB, 144, 512), F32),
            pltpu.VMEM((GB, 256, 512), BF), pltpu.VMEM((GB, 256, 512), BF),
            pltpu.VMEM((GM, 8, 512), F32), pltpu.VMEM((GM, 8, 512), F32),
            pltpu.VMEM((GM, 8, 512), F32), pltpu.VMEM((GM, 8, 512), F32),
            pltpu.SemaphoreType.DMA((NC,)),
            pltpu.SemaphoreType.DMA((4,)),
            pltpu.SemaphoreType.DMA((NC,)),
        ],
        compiler_params=pltpu.CompilerParams(vmem_limit_bytes=100 * 1024 * 1024),
    )(ba, bb, A_x.reshape(S, D), A_wqkv, A_wo, B_wqkv, B_wo)
    return out.reshape(1, S, D)
```

```python
import math

import jax
import jax.numpy as jnp
import numpy as np
from jax import lax
import jax.experimental.pallas as pl
import jax.experimental.pallas.tpu as pltpu

S = 2048
D = 1024
H = 32
DH = 32
NG = D // 128
TQ = 128
NT = S // TQ
PAD = 256
GA = 4
GB = 8
GM = max(GA, GB)
ORDER_A = '01p2q3'
ORDER_B = '01p2q3'
TC = 512
NC = S // TC
NEG = -1e9
QSCALE = (DH ** -0.5) * math.log2(math.e)
EPS = 1e-5
BF = jnp.bfloat16
F32 = jnp.float32
NT_DIMS = (((1,), (1,)), ((), ()))


def _bias_tables():
    k = np.arange(384)[:, None] - 256
    q = np.arange(128)[None, :]
    a = []
    for t in range(3):
        ok = (q - k >= 0) & (q - k < 256) & (k + t * 128 >= 0)
        a.append(np.where(ok, 0.0, NEG))
    k = np.arange(144)[:, None] - 16
    b = []
    for t in range(2):
        d = q - k
        ok = (d >= 0) & (d <= 14) & (d % 2 == 0) & (k + t * 128 >= 0)
        b.append(np.where(ok, 0.0, NEG))
    return np.stack(a).astype(np.float32), np.stack(b).astype(np.float32)


def _kernel(ba_ref, bb_ref, x_hbm, wa_hbm, woa_hbm, wb_hbm, wob_hbm, out_hbm,
            xin, xr, w, wo, qT, kk, vT, oo, stage,
            sa0, sa1, pa0, pa1, sb0, sb1, pb0, pb1, m0, m1, l0, l1, sem_x, sem_w, sem_a, sem_o):
    def x_copy(c):
        return pltpu.make_async_copy(x_hbm.at[pl.ds(c * TC, TC)], xin.at[pl.ds(c * TC, TC)], sem_x.at[c])

    CB = 512
    wa_cols = [t * D + b * CB for b in range(D // CB) for t in range(3)]
    wa_copies = [
        pltpu.make_async_copy(wa_hbm.at[:, pl.ds(c0, CB)], w.at[0, :, pl.ds(c0, CB)], sem_a.at[n])
        for n, c0 in enumerate(wa_cols)]
    w_copies = [
        pltpu.make_async_copy(woa_hbm, wo.at[0], sem_w.at[0]),
        pltpu.make_async_copy(wb_hbm, w.at[1], sem_w.at[1]),
        pltpu.make_async_copy(wob_hbm, wo.at[1], sem_w.at[2]),
    ]
    x_copy(0).start()
    for cp in wa_copies:
        cp.start()

    for g in range(NG):
        kk[g, 0:PAD, :] = jnp.zeros((PAD, 128), BF)
        for t in range(PAD // 128):
            vT[t, g] = jnp.zeros((128, 128), BF)

    def project(c, x, wi, hook=lambda n: None):
        m = jnp.mean(x, axis=-1, keepdims=True)
        xc = x - m
        v = jnp.mean(xc * xc, axis=-1, keepdims=True)
        ln = (xc * lax.rsqrt(v + EPS)).astype(BF)
        for b in range(D // 512):
            hook(3 * b)
            q = jnp.dot(ln, w[wi, :, b * 512:(b + 1) * 512], preferred_element_type=F32)
            q = (q * QSCALE).astype(BF)
            for j in range(4):
                for t in range(TC // 128):
                    qT[c * (TC // 128) + t, b * 4 + j] = q[t * 128:(t + 1) * 128, j * 128:(j + 1) * 128].T
            hook(3 * b + 1)
            k = jnp.dot(ln, w[wi, :, D + b * 512:D + (b + 1) * 512], preferred_element_type=F32).astype(BF)
            for j in range(4):
                kk[b * 4 + j, pl.ds(pl.multiple_of(PAD + c * TC, 128), TC), :] = k[:, j * 128:(j + 1) * 128]
            hook(3 * b + 2)
            vv = jnp.dot(ln, w[wi, :, 2 * D + b * 512:2 * D + (b + 1) * 512], preferred_element_type=F32).astype(BF)
            for j in range(4):
                for t in range(TC // 128):
                    vT[2 + c * (TC // 128) + t, b * 4 + j] = vv[t * 128:(t + 1) * 128, j * 128:(j + 1) * 128].T

    def masked_q(i, g):
        q4 = qT[i, g]
        z = jnp.zeros((32, 128), BF)
        cols = []
        for h in range(4):
            cols.append(jnp.concatenate([q4[32 * h:32 * h + 32] if hh == h else z for hh in range(4)], axis=0))
        return jnp.concatenate(cols, axis=1)

    def attention(nk, G, bias_ref, Sb, Pb, Mb, Lb):
        is_a = nk == 384
        nb = NT * NG // G
        prow = 0 if is_a else 112

        def qk(j, b, u):
            n = j * G + u
            i, g = n // NG, n % NG
            k4 = kk[g, pl.ds(pl.multiple_of(i * 128 + PAD + 128 - nk, 16), nk), :]
            s = jnp.dot(k4, masked_q(i, g), preferred_element_type=F32)
            bi = jnp.minimum(i, 2 if is_a else 1)
            ms = [None] * 4
            for r in range(0, nk, 8):
                bias = bias_ref[bi, r:r + 8, :]
                for h in range(4):
                    c = s[r:r + 8, h * 128:(h + 1) * 128] + bias
                    Sb[b][u, r:r + 8, h * 128:(h + 1) * 128] = c
                    ms[h] = c if ms[h] is None else jnp.maximum(ms[h], c)
            for h in range(4):
                Mb[b][u, :, h * 128:(h + 1) * 128] = jnp.broadcast_to(
                    jnp.max(ms[h], axis=0, keepdims=True), (8, 128))

        def ex(b, u, hs):
            for h in hs:
                cs = slice(h * 128, (h + 1) * 128)
                m = Mb[b][u, :, cs]
                l = None
                for r in range(0, nk, 16):
                    pa = jnp.exp2(Sb[b][u, r:r + 8, cs] - m)
                    pb = jnp.exp2(Sb[b][u, r + 8:r + 16, cs] - m)
                    t = pa + pb
                    l = t if l is None else l + t
                    Pb[b][u, prow + r:prow + r + 16, cs] = jnp.concatenate([pa, pb], axis=0).astype(BF)
                Lb[b][u, :, cs] = jnp.broadcast_to(
                    pltpu.reciprocal(jnp.sum(l, axis=0, keepdims=True), approx=False), (8, 128))

        def pv(j, b, u):
            n = j * G + u
            i, g = n // NG, n % NG
            t0, npr = (0, 384) if is_a else (1, 256)
            outs = []
            for h in range(4):
                cs = slice(h * 128, (h + 1) * 128)
                vt = jnp.concatenate([vT[i + t, g, 32 * h:32 * h + 32, :] for t in range(t0, 3)], axis=1)
                o = jnp.dot(vt, Pb[b][u, 0:npr, cs], preferred_element_type=F32)
                outs.append(o * Lb[b][u, 0:1, cs])
            oo[g, pl.ds(pl.multiple_of(i * 128, 128), 128), :] = jnp.concatenate(outs, axis=0).astype(BF).T

        if not is_a:
            for b in range(2):
                for u in range(G):
                    Pb[b][u, 0:prow, :] = jnp.zeros((prow, 512), BF)

        def step(j, b, p=True, e=True, q=True):
            for u in range(G):
                for ch in (ORDER_A if is_a else ORDER_B):
                    if ch == 'p' and p:
                        pv(j - 1, 1 - b, u)
                    if ch.isdigit() and e:
                        ex(b, u, [int(ch)])
                    if ch == 'q' and q:
                        qk(j + 1, 1 - b, u)

        step(-1, 1, p=False, e=False)
        step(0, 0, p=False)

        def body(j, _):
            pl.when(j % 2 == 1)(lambda: step(j, 1))
            pl.when(j % 2 == 0)(lambda: step(j, 0))
            return 0
        lax.fori_loop(1, nb - 1, body, 0)
        step(nb - 1, 1, q=False)
        step(nb, 0, e=False, q=False)

    def attn_a():
        attention(384, GA, ba_ref, (sa0, sa1), (pa0, pa1), (m0, m1), (l0, l1))

    def attn_b():
        attention(144, GB, bb_ref, (sb0, sb1), (pb0, pb1), (m0, m1), (l0, l1))

    def outproj(c, wi):
        r0 = pl.multiple_of(c * TC, TC)
        o = jnp.concatenate([oo[g, pl.ds(r0, TC), :] for g in range(NG)], axis=1)
        return xr[pl.ds(r0, TC), :] + jnp.dot(o, wo[wi], preferred_element_type=F32)

    def first(c, hook):
        x_copy(c).wait()
        r0 = pl.multiple_of(c * TC, TC)
        x = xin[pl.ds(r0, TC), :].astype(F32)
        xr[pl.ds(r0, TC), :] = x
        project(c, x, 0, hook)

    def hook0(n):
        wa_copies[n].wait()
        if n == 1:
            for c in range(1, NC):
                x_copy(c).start()
        if n == 5:
            for cp in w_copies:
                cp.start()
    first(0, hook0)
    lax.fori_loop(1, NC, lambda c, _: (first(c, lambda n: None), 0)[1], 0)
    for cp in w_copies:
        cp.wait()

    def mid(wi):
        def body(c, _):
            x = outproj(c, wi)
            xr[pl.ds(pl.multiple_of(c * TC, TC), TC), :] = x
            project(c, x, 1 - wi)
            return 0
        return body

    def pair(p, _):
        attn_a()
        lax.fori_loop(0, NC, mid(0), 0)
        attn_b()

        @pl.when(p == 0)
        def _():
            lax.fori_loop(0, NC, mid(1), 0)
        return 0
    lax.fori_loop(0, 2, pair, 0)

    def out_copy(c):
        return pltpu.make_async_copy(stage.at[c], out_hbm.at[pl.ds(c * TC, TC)], sem_o.at[c])

    def last(c, _):
        stage[c] = outproj(c, 1).astype(BF)
        out_copy(c).start()
        return 0
    lax.fori_loop(0, NC, last, 0)
    for c in range(NC):
        out_copy(c).wait()


@jax.jit
def pallas_interleave_layers__sliding_block__sliding_local_dilated__prompt_kernel(
    A_x, A_wqkv, A_wo, B_x, B_wqkv, B_wo,
):
    ba, bb = _bias_tables()
    any_spec = pl.BlockSpec(memory_space=pl.ANY)
    vm = pl.BlockSpec(memory_space=pltpu.VMEM)
    out = pl.pallas_call(
        _kernel,
        out_shape=jax.ShapeDtypeStruct((S, D), BF),
        in_specs=[vm, vm] + [any_spec] * 5,
        out_specs=any_spec,
        scratch_shapes=[
            pltpu.VMEM((S, D), BF),
            pltpu.VMEM((S, D), F32),
            pltpu.VMEM((2, D, 3 * D), BF),
            pltpu.VMEM((2, D, D), BF),
            pltpu.VMEM((NT, NG, 128, 128), BF),
            pltpu.VMEM((NG, S + PAD, 128), BF),
            pltpu.VMEM((NT + 2, NG, 128, 128), BF),
            pltpu.VMEM((NG, S, 128), BF),
            pltpu.VMEM((NC, TC, D), BF),
            pltpu.VMEM((GA, 384, 512), F32), pltpu.VMEM((GA, 384, 512), F32),
            pltpu.VMEM((GA, 384, 512), BF), pltpu.VMEM((GA, 384, 512), BF),
            pltpu.VMEM((GB, 144, 512), F32), pltpu.VMEM((GB, 144, 512), F32),
            pltpu.VMEM((GB, 256, 512), BF), pltpu.VMEM((GB, 256, 512), BF),
            pltpu.VMEM((GM, 8, 512), F32), pltpu.VMEM((GM, 8, 512), F32),
            pltpu.VMEM((GM, 8, 512), F32), pltpu.VMEM((GM, 8, 512), F32),
            pltpu.SemaphoreType.DMA((NC,)),
            pltpu.SemaphoreType.DMA((3,)),
            pltpu.SemaphoreType.DMA((6,)),
            pltpu.SemaphoreType.DMA((NC,)),
        ],
        compiler_params=pltpu.CompilerParams(vmem_limit_bytes=100 * 1024 * 1024),
    )(ba, bb, A_x.reshape(S, D), A_wqkv, A_wo, B_wqkv, B_wo)
    return out.reshape(1, S, D)
```
